```python
import os as _os
_os.environ.setdefault("JAX_PLATFORMS", "cpu")
import jax
import jax.numpy as jnp

def _softmax(x, axis=-1):
    return jax.nn.softmax(x, axis=axis)
def _gelu(x):
    return jax.nn.gelu(x, approximate=True)
def _silu(x):
    return jax.nn.silu(x)
def _sigmoid(x):
    return jax.nn.sigmoid(x)
def _layernorm(x, axis=-1, eps=1e-5):
    m = jnp.mean(x, axis=axis, keepdims=True)
    v = jnp.var(x, axis=axis, keepdims=True)
    return (x - m) / jnp.sqrt(v + eps)
def _scatter_add(tgt, idx, src, axis=0):
    return tgt.at[idx].add(src)
def _segment_sum(src, seg, n):
    return jax.ops.segment_sum(src, seg, n)
class _Rng:
    def __init__(self, key):
        self._k = key
    def _next(self):
        self._k, sub = jax.random.split(self._k)
        return sub
    def normal(self, shape):
        return jax.random.normal(self._next(), shape, dtype=jnp.bfloat16)
    def randint(self, lo, hi, shape):
        return jax.random.randint(self._next(), shape, lo, hi, dtype=jnp.int32)
    def uniform(self, shape, lo=0.0, hi=1.0):
        return jax.random.uniform(self._next(), shape, jnp.bfloat16, lo, hi)
    def permutation(self, n):
        return jax.random.permutation(self._next(), n)


kernel_name = 'concat_heads__grouped_kv_mqa__sliding_block__prompt'

def setup_inputs():
    _rng = _Rng(jax.random.key(int.from_bytes(__import__("os").urandom(4), "little")))
    _w = (lambda a: (lambda t: t.astype(jnp.bfloat16) if jnp.issubdtype(t.dtype, jnp.floating) else t)(jnp.asarray(a)))
    def _A_setup():
        B, S, D, H = 1, 2048, 1024, 32
        Dh = D // H
        return {
            "x": _w((lambda *s: _rng.normal(s) * 0.05)(B, S, D)),
            "wq": _w((lambda *s: _rng.normal(s) * 1.6)(D, H * Dh)),
            "wk": _w((lambda *s: _rng.normal(s) * 1.6)(D, Dh)),
            "wv": _w((lambda *s: _rng.normal(s) * 0.1)(D, Dh)),
            "wo": _w((lambda *s: _rng.normal(s) * 0.1)(H * Dh, D)),
        }
    _A_in = _A_setup()

    def _B_setup():
        B, S, D = 1, 2048, 1024
        return {
            "x": _w((lambda *s: _rng.normal(s) * 0.2)(B, S, D)),
            "wqkv": _w((lambda *s: _rng.normal(s) * 0.2)(D, 3 * D)),
            "wo": _w((lambda *s: _rng.normal(s) * 0.05)(D, D)),
        }
    _B_in = _B_setup()

    return {
        "A_x": _A_in["x"],
        "A_wq": _A_in["wq"],
        "A_wk": _A_in["wk"],
        "A_wv": _A_in["wv"],
        "A_wo": _A_in["wo"],
        "B_x": _B_in["x"],
        "B_wqkv": _B_in["wqkv"],
        "B_wo": _B_in["wo"],
    }

def reference(A_x, A_wq, A_wk, A_wv, A_wo, B_x, B_wqkv, B_wo):
    def _A_ref(x, wq, wk, wv, wo):
        B, S, D = x.shape
        H = 32
        Dh = D // H
        q = (lambda x, *d: x.transpose(*d))((x @ wq).reshape(B, S, H, Dh), 0, 2, 1, 3)
        k = x @ wk
        v = x @ wv
        scores = jnp.einsum("bhqd,bkd->bhqk", q, k) * (Dh ** -0.5)
        p = _softmax(scores, axis=-1)
        o = jnp.einsum("bhqk,bkd->bhqd", p, v)
        return (lambda x, *d: x.transpose(*d))(o, 0, 2, 1, 3).reshape(B, S, H * Dh) @ wo

    def _B_ref(x, wqkv, wo):
        B, S, D = x.shape
        H = 32; Dh = D // H; W = 256
        qkv = (lambda x, *d: x.transpose(*d))((x @ wqkv).reshape(B, S, 3, H, Dh), 2, 0, 3, 1, 4)
        q, k, v = qkv[0], qkv[1], qkv[2]
        scores = jnp.einsum("bhqd,bhkd->bhqk", q, k) * (Dh ** -0.5)
        idx = jnp.arange(S)
        mask = (idx[:, None] - idx[None, :] >= 0) & (idx[:, None] - idx[None, :] < W)
        scores = jnp.where(mask[None, None], scores, -1e9)
        p = _softmax(scores, axis=-1)
        o = jnp.einsum("bhqk,bhkd->bhqd", p, v)
        return (lambda x, *d: x.transpose(*d))(o, 0, 2, 1, 3).reshape(B, S, D) @ wo

    a = _A_ref(A_x, A_wq, A_wk, A_wv, A_wo)
    b = _B_ref(B_x, B_wqkv, B_wo)
    return jnp.concatenate([a, b], axis=-1)
```

```python
import math

import jax
import jax.numpy as jnp
import jax.experimental.pallas as pl
import jax.experimental.pallas.tpu as pltpu

S = 2048
D = 1024
H = 32
DH = 32
W = 256
BQ = 512
CK = 128
QB = 128
KW = W + QB
SCALE = (DH ** -0.5) * math.log2(math.e)
NEG = -1e30

F32 = jnp.float32
BF16 = jnp.bfloat16


def _dot(a, b):
    return jnp.dot(a, b, preferred_element_type=F32)


def _kernel(xa_ref, wqa_ref, wkva_ref, woa_ref, xb_ref, wqkvb_ref, wob_ref,
            out_ref,
            ka_ref, vat_ref, qt_ref, ot_ref, sa_ref, sb_ref, kb_ref, vbt_ref):
    i = pl.program_id(0)
    nck = S // CK

    @pl.when(i == 0)
    def _():
        kv = _dot(xa_ref[...], wkva_ref[...])
        ka_ref[...] = kv[:, 0:DH].astype(BF16)
        vat_ref[...] = kv.T[DH:2 * DH, :].astype(BF16)

    row0 = pl.multiple_of(i * BQ, BQ)
    q = _dot(xa_ref[pl.ds(row0, BQ), :], wqa_ref[...]) * SCALE
    qt_ref[...] = q.T.astype(BF16)

    def qk_chunk(qh, buf, c, m_next):
        s = _dot(ka_ref[c * CK:(c + 1) * CK, :], qh)
        buf[c * CK:(c + 1) * CK, :] = s
        return jnp.maximum(m_next, jnp.max(s, axis=0, keepdims=True))

    def pv_chunk(buf, c, m, l, o):
        p = jnp.exp2(buf[c * CK:(c + 1) * CK, :] - m)
        l = l + jnp.sum(p, axis=0, keepdims=True)
        o = o + _dot(vat_ref[:, c * CK:(c + 1) * CK], p.astype(BF16))
        return l, o

    def stage(h, m, cur, nxt, do_qk=True):
        off = pl.multiple_of(h * DH, DH)
        m_next = jnp.full((1, BQ), -jnp.inf, F32)
        if do_qk:
            offn = pl.multiple_of((h + 1) * DH, DH)
            qn = qt_ref[pl.ds(offn, DH), :]
        l = jnp.zeros((1, BQ), F32)
        o = jnp.zeros((DH, BQ), F32)
        for c in range(nck):
            if do_qk:
                m_next = qk_chunk(qn, nxt, c, m_next)
            l, o = pv_chunk(cur, c, m, l, o)
        ot_ref[pl.ds(off, DH), :] = o / l
        return m_next

    q0 = qt_ref[0:DH, :]
    m0 = jnp.full((1, BQ), -jnp.inf, F32)
    for c in range(nck):
        m0 = qk_chunk(q0, sa_ref, c, m0)

    def pair(j, m):
        h = 2 * j
        m = stage(h, m, sa_ref, sb_ref)
        m = stage(h + 1, m, sb_ref, sa_ref)
        return m

    m = jax.lax.fori_loop(0, H // 2 - 1, pair, m0)
    m = stage(H - 2, m, sa_ref, sb_ref)
    stage(H - 1, m, sb_ref, sa_ref, do_qk=False)

    oa = ot_ref[...].T.astype(BF16)
    out_ref[:, 0:D] = _dot(oa, woa_ref[...]).astype(out_ref.dtype)

    xb = xb_ref[...]
    qb = _dot(xb, wqkvb_ref[:, 0:D]) * SCALE
    qt_ref[...] = qb.T.astype(BF16)
    kb_ref[pl.ds(row0, BQ), :] = _dot(xb, wqkvb_ref[:, D:2 * D]).astype(BF16)
    vb = _dot(xb, wqkvb_ref[:, 2 * D:3 * D])
    vbt_ref[:, pl.ds(row0, BQ)] = vb.T.astype(BF16)

    rowgrp = jax.lax.broadcasted_iota(jnp.int32, (4 * DH, QB), 0) // DH
    kiota = jax.lax.broadcasted_iota(jnp.int32, (KW, QB), 0)
    qiota = jax.lax.broadcasted_iota(jnp.int32, (KW, QB), 1)

    for t in range(BQ // QB):
        n = i * (BQ // QB) + t
        start = pl.multiple_of(jnp.maximum(n - 2, 0) * QB, QB)
        diff = (n * QB + qiota) - (start + kiota)
        mask1 = jnp.logical_and(diff >= 0, diff < W)
        mask = jnp.concatenate([mask1] * 4, axis=1)
        for g in range(H // 4):
            qg = qt_ref[g * 4 * DH:(g + 1) * 4 * DH, t * QB:(t + 1) * QB]
            zero = jnp.zeros_like(qg)
            qm = jnp.concatenate(
                [jnp.where(rowgrp == j, qg, zero) for j in range(4)], axis=1)
            kwin = kb_ref[pl.ds(start, KW), g * 4 * DH:(g + 1) * 4 * DH]
            s = _dot(kwin, qm)
            s = jnp.where(mask, s, NEG)
            mx = jnp.max(s, axis=0, keepdims=True)
            p = jnp.exp2(s - mx)
            l = jnp.sum(p, axis=0, keepdims=True)
            pb = p.astype(BF16)
            for j in range(4):
                h = 4 * g + j
                vwin = vbt_ref[h * DH:(h + 1) * DH, pl.ds(start, KW)]
                o = _dot(vwin, pb[:, j * QB:(j + 1) * QB])
                ot_ref[h * DH:(h + 1) * DH, t * QB:(t + 1) * QB] = o / l[:, j * QB:(j + 1) * QB]

    ob = ot_ref[...].T.astype(BF16)
    out_ref[:, D:2 * D] = _dot(ob, wob_ref[...]).astype(out_ref.dtype)


@jax.jit
def pallas_concat_heads__grouped_kv_mqa__sliding_block__prompt_kernel(
    A_x: jax.Array,
    A_wq: jax.Array,
    A_wk: jax.Array,
    A_wv: jax.Array,
    A_wo: jax.Array,
    B_x: jax.Array,
    B_wqkv: jax.Array,
    B_wo: jax.Array,
):
    xa = A_x.reshape(S, D)
    xb = B_x.reshape(S, D)
    wkva = jnp.pad(jnp.concatenate([A_wk, A_wv], axis=1), ((0, 0), (0, 128 - 2 * DH)))

    const = lambda i: (0, 0)
    out = pl.pallas_call(
        _kernel,
        grid=(S // BQ,),
        in_specs=[
            pl.BlockSpec((S, D), const),
            pl.BlockSpec((D, D), const),
            pl.BlockSpec((D, 128), const),
            pl.BlockSpec((D, D), const),
            pl.BlockSpec((BQ, D), lambda i: (i, 0)),
            pl.BlockSpec((D, 3 * D), const),
            pl.BlockSpec((D, D), const),
        ],
        out_specs=pl.BlockSpec((BQ, 2 * D), lambda i: (i, 0)),
        out_shape=jax.ShapeDtypeStruct((S, 2 * D), BF16),
        scratch_shapes=[
            pltpu.VMEM((S, DH), BF16),
            pltpu.VMEM((DH, S), BF16),
            pltpu.VMEM((D, BQ), BF16),
            pltpu.VMEM((D, BQ), F32),
            pltpu.VMEM((S, BQ), F32),
            pltpu.VMEM((S, BQ), F32),
            pltpu.VMEM((S, D), BF16),
            pltpu.VMEM((D, S), BF16),
        ],
        compiler_params=pltpu.CompilerParams(
            dimension_semantics=("arbitrary",),
            vmem_limit_bytes=100 * 1024 * 1024,
        ),
    )(xa, A_wq, wkva, A_wo, xb, B_wqkv, B_wo)
    return out.reshape(1, S, 2 * D)
```

```python
import math

import jax
import jax.numpy as jnp
import jax.experimental.pallas as pl
import jax.experimental.pallas.tpu as pltpu

S = 2048
D = 1024
H = 32
DH = 32
W = 256
BQ = 512
CK = 128
QB = 128
KW = W + QB
SCALE = (DH ** -0.5) * math.log2(math.e)
NEG = -1e30

F32 = jnp.float32
BF16 = jnp.bfloat16


def _dot(a, b):
    return jnp.dot(a, b, preferred_element_type=F32)


def _kernel(xa_ref, wqa_ref, wkva_ref, woa_ref, xb_ref, wqkvb_ref, wob_ref,
            out_ref,
            ka_ref, vat_ref, qt_ref, ot_ref, sa_ref, sb_ref, kb_ref, vbt_ref):
    i = pl.program_id(0)
    nck = S // CK

    @pl.when(i == 0)
    def _():
        kv = _dot(xa_ref[...], wkva_ref[...])
        ka_ref[...] = kv[:, 0:DH].astype(BF16)
        vat_ref[...] = kv.T[DH:2 * DH, :].astype(BF16)

    row0 = pl.multiple_of(i * BQ, BQ)
    q = _dot(xa_ref[pl.ds(row0, BQ), :], wqa_ref[...]) * SCALE
    qt_ref[...] = q.T.astype(BF16)

    def qk_chunk(qh, buf, c, m_next):
        s = _dot(ka_ref[c * CK:(c + 1) * CK, :], qh)
        buf[c * CK:(c + 1) * CK, :] = s
        return jnp.maximum(m_next, jnp.max(s, axis=0, keepdims=True))

    def pv_chunk(buf, c, m, l, o):
        p = jnp.exp2(buf[c * CK:(c + 1) * CK, :] - m)
        l = l + jnp.sum(p, axis=0, keepdims=True)
        o = o + _dot(vat_ref[:, c * CK:(c + 1) * CK], p.astype(BF16))
        return l, o

    def stage(h, m, cur, nxt, do_qk=True):
        off = pl.multiple_of(h * DH, DH)
        m_next = jnp.full((1, BQ), -jnp.inf, F32)
        if do_qk:
            offn = pl.multiple_of((h + 1) * DH, DH)
            qn = qt_ref[pl.ds(offn, DH), :]
        l = jnp.zeros((1, BQ), F32)
        o = jnp.zeros((DH, BQ), F32)
        for c in range(nck):
            if do_qk:
                m_next = qk_chunk(qn, nxt, c, m_next)
            l, o = pv_chunk(cur, c, m, l, o)
        ot_ref[pl.ds(off, DH), :] = o / l
        return m_next

    q0 = qt_ref[0:DH, :]
    m0 = jnp.full((1, BQ), -jnp.inf, F32)
    for c in range(nck):
        m0 = qk_chunk(q0, sa_ref, c, m0)

    def pair(j, m):
        h = 2 * j
        m = stage(h, m, sa_ref, sb_ref)
        m = stage(h + 1, m, sb_ref, sa_ref)
        return m

    m = jax.lax.fori_loop(0, H // 2 - 1, pair, m0)
    m = stage(H - 2, m, sa_ref, sb_ref)
    stage(H - 1, m, sb_ref, sa_ref, do_qk=False)

    oa = ot_ref[...].T.astype(BF16)
    out_ref[:, 0:D] = _dot(oa, woa_ref[...]).astype(out_ref.dtype)

    xb = xb_ref[...]
    qb = _dot(xb, wqkvb_ref[:, 0:D]) * SCALE
    qt_ref[...] = qb.T.astype(BF16)
    kb_ref[pl.ds(row0, BQ), :] = _dot(xb, wqkvb_ref[:, D:2 * D]).astype(BF16)
    vb = _dot(xb, wqkvb_ref[:, 2 * D:3 * D])
    vbt_ref[:, pl.ds(row0, BQ)] = vb.T.astype(BF16)

    rowgrp = jax.lax.broadcasted_iota(jnp.int32, (4 * DH, QB), 0) // DH
    kiota = jax.lax.broadcasted_iota(jnp.int32, (QB, QB), 0)
    qiota = jax.lax.broadcasted_iota(jnp.int32, (QB, QB), 1)
    NG = H // 4
    NU = (BQ // QB) * NG
    NC = KW // QB

    def unit_coords(u):
        t = u // NG
        g = u % NG
        n = i * (BQ // QB) + t
        start = jnp.maximum(n - 2, 0) * QB
        return t, g, n, start

    def b_setup(u):
        t, g, n, start = unit_coords(u)
        goff = pl.multiple_of(g * 4 * DH, 4 * DH)
        qg = qt_ref[pl.ds(goff, 4 * DH), pl.ds(pl.multiple_of(t * QB, QB), QB)]
        zero = jnp.zeros_like(qg)
        qm = jnp.concatenate(
            [jnp.where(rowgrp == j, qg, zero) for j in range(4)], axis=1)
        return qm

    def b_qk_chunk(u, qm, buf, c, m):
        t, g, n, start = unit_coords(u)
        goff = pl.multiple_of(g * 4 * DH, 4 * DH)
        koff = pl.multiple_of(start + c * QB, QB)
        diff = (n * QB + qiota) - (koff + kiota)
        mask1 = jnp.logical_and(diff >= 0, diff < W)
        mask = jnp.concatenate([mask1] * 4, axis=1)
        s = _dot(kb_ref[pl.ds(koff, QB), pl.ds(goff, 4 * DH)], qm)
        s = jnp.where(mask, s, NEG)
        buf[c * QB:(c + 1) * QB, :] = s
        cm = jnp.max(s, axis=0, keepdims=True)
        return cm if m is None else jnp.maximum(m, cm)

    def b_pv_chunk(u, buf, c, m, l, os_):
        t, g, n, start = unit_coords(u)
        koff = pl.multiple_of(start + c * QB, QB)
        p = jnp.exp2(buf[c * QB:(c + 1) * QB, :] - m)
        cl = jnp.sum(p, axis=0, keepdims=True)
        l = cl if l is None else l + cl
        pb = p.astype(BF16)
        new_os = []
        for j in range(4):
            hoff = pl.multiple_of((4 * g + j) * DH, DH)
            oj = _dot(vbt_ref[pl.ds(hoff, DH), pl.ds(koff, QB)], pb[:, j * QB:(j + 1) * QB])
            new_os.append(oj if os_ is None else os_[j] + oj)
        return l, new_os

    def b_stage(u, m, cur, nxt, do_qk=True):
        m_next = None
        if do_qk:
            qm = b_setup(u + 1)
        l = None
        os_ = None
        for c in range(NC):
            if do_qk:
                m_next = b_qk_chunk(u + 1, qm, nxt, c, m_next)
            l, os_ = b_pv_chunk(u, cur, c, m, l, os_)
        t, g, n, start = unit_coords(u)
        toff = pl.multiple_of(t * QB, QB)
        for j in range(4):
            hoff = pl.multiple_of((4 * g + j) * DH, DH)
            ot_ref[pl.ds(hoff, DH), pl.ds(toff, QB)] = os_[j] / l[:, j * QB:(j + 1) * QB]
        return m_next

    qm0 = b_setup(0)
    mb = None
    for c in range(NC):
        mb = b_qk_chunk(0, qm0, sa_ref, c, mb)

    def b_pair(j, m):
        u = 2 * j
        m = b_stage(u, m, sa_ref, sb_ref)
        m = b_stage(u + 1, m, sb_ref, sa_ref)
        return m

    mb = jax.lax.fori_loop(0, NU // 2 - 1, b_pair, mb)
    mb = b_stage(NU - 2, mb, sa_ref, sb_ref)
    b_stage(NU - 1, mb, sb_ref, sa_ref, do_qk=False)

    ob = ot_ref[...].T.astype(BF16)
    out_ref[:, D:2 * D] = _dot(ob, wob_ref[...]).astype(out_ref.dtype)


@jax.jit
def pallas_concat_heads__grouped_kv_mqa__sliding_block__prompt_kernel(
    A_x: jax.Array,
    A_wq: jax.Array,
    A_wk: jax.Array,
    A_wv: jax.Array,
    A_wo: jax.Array,
    B_x: jax.Array,
    B_wqkv: jax.Array,
    B_wo: jax.Array,
):
    xa = A_x.reshape(S, D)
    xb = B_x.reshape(S, D)
    wkva = jnp.pad(jnp.concatenate([A_wk, A_wv], axis=1), ((0, 0), (0, 128 - 2 * DH)))

    const = lambda i: (0, 0)
    out = pl.pallas_call(
        _kernel,
        grid=(S // BQ,),
        in_specs=[
            pl.BlockSpec((S, D), const),
            pl.BlockSpec((D, D), const),
            pl.BlockSpec((D, 128), const),
            pl.BlockSpec((D, D), const),
            pl.BlockSpec((BQ, D), lambda i: (i, 0)),
            pl.BlockSpec((D, 3 * D), const),
            pl.BlockSpec((D, D), const),
        ],
        out_specs=pl.BlockSpec((BQ, 2 * D), lambda i: (i, 0)),
        out_shape=jax.ShapeDtypeStruct((S, 2 * D), BF16),
        scratch_shapes=[
            pltpu.VMEM((S, DH), BF16),
            pltpu.VMEM((DH, S), BF16),
            pltpu.VMEM((D, BQ), BF16),
            pltpu.VMEM((D, BQ), F32),
            pltpu.VMEM((S, BQ), F32),
            pltpu.VMEM((S, BQ), F32),
            pltpu.VMEM((S, D), BF16),
            pltpu.VMEM((D, S), BF16),
        ],
        compiler_params=pltpu.CompilerParams(
            dimension_semantics=("arbitrary",),
            vmem_limit_bytes=100 * 1024 * 1024,
        ),
    )(xa, A_wq, wkva, A_wo, xb, B_wqkv, B_wo)
    return out.reshape(1, S, 2 * D)
```

```python
import math

import jax
import jax.numpy as jnp
import jax.experimental.pallas as pl
import jax.experimental.pallas.tpu as pltpu

S = 2048
D = 1024
H = 32
DH = 32
W = 256
BQ = 512
CK = 128
NCK = S // CK
QB = 128
KW = W + QB
NC = KW // QB
NG = H // 4
NT = BQ // QB
KA = 2
KB = 2
PR = 256
SCALE = (DH ** -0.5) * math.log2(math.e)
NEG = -1e30

F32 = jnp.float32
BF16 = jnp.bfloat16


def _dot(a, b):
    return jnp.dot(a, b, preferred_element_type=F32)


def _kernel(xa_hbm, wqa_hbm, wkva_hbm, woa_hbm, xb_hbm, wqkvb_hbm, wob_hbm,
            out_ref,
            xa_ref, wqa_ref, wkva_ref, woa_ref, xb_ref, wqkvb_ref, wob_ref, sems,
            ka_ref, vat_ref, qt_ref, ot_ref, sa_ref, sb_ref, kb_ref, vbt_ref, qm_ref):
    i = pl.program_id(0)
    row0 = pl.multiple_of(i * BQ, BQ)
    bufs = (sa_ref, sb_ref)

    cp_xa0 = pltpu.make_async_copy(xa_hbm.at[0:BQ, :], xa_ref.at[0:BQ, :], sems.at[0])
    cp_wqa = pltpu.make_async_copy(wqa_hbm, wqa_ref, sems.at[1])
    cp_xa1 = pltpu.make_async_copy(xa_hbm.at[BQ:S, :], xa_ref.at[BQ:S, :], sems.at[2])
    cp_wkva = pltpu.make_async_copy(wkva_hbm, wkva_ref, sems.at[3])
    cp_woa = pltpu.make_async_copy(woa_hbm, woa_ref, sems.at[4])
    cp_wqkvb = pltpu.make_async_copy(wqkvb_hbm, wqkvb_ref, sems.at[5])
    cp_wob = pltpu.make_async_copy(wob_hbm, wob_ref, sems.at[6])
    cp_xb = pltpu.make_async_copy(xb_hbm.at[pl.ds(row0, BQ), :], xb_ref, sems.at[7])

    @pl.when(i == 0)
    def _():
        cp_xa0.start()
        cp_wqa.start()
        cp_xa1.start()
        cp_wkva.start()
        cp_woa.start()

    cp_xb.start()

    @pl.when(i == 0)
    def _():
        cp_wqkvb.start()
        cp_wob.start()
        def zfill(r, c):
            roff = pl.multiple_of(r * 256, 256)
            sa_ref[pl.ds(roff, 256), :] = jnp.zeros((256, BQ), F32)
            sb_ref[pl.ds(roff, 256), :] = jnp.zeros((256, BQ), F32)
            return c
        jax.lax.fori_loop(0, S // 256, zfill, 0)
        cp_xa0.wait()
        cp_wqa.wait()

    q = _dot(xa_ref[pl.ds(row0, BQ), :], wqa_ref[...]) * SCALE
    qt_ref[...] = q.T.astype(BF16)

    @pl.when(i == 0)
    def _():
        cp_xa1.wait()
        cp_wkva.wait()
        def kv_proj(r, c):
            roff = pl.multiple_of(r * 512, 512)
            kv = _dot(xa_ref[pl.ds(roff, 512), :], wkva_ref[...])
            ka_ref[pl.ds(roff, 512), :] = kv[:, 0:DH].astype(BF16)
            vat_ref[:, pl.ds(roff, 512)] = kv.T[DH:2 * DH, :].astype(BF16)
            return c
        jax.lax.fori_loop(0, S // 512, kv_proj, 0)

    def qk_chunk(qh, buf, c, m8):
        s = _dot(ka_ref[c * CK:(c + 1) * CK, :], qh)
        buf[c * CK:(c + 1) * CK, :] = s
        cm = jnp.max(s.reshape(CK // 8, 8, BQ), axis=0)
        return cm if m8 is None else jnp.maximum(m8, cm)

    def pv_chunk(buf, c, m, l8, o):
        if l8 is not None:
            m = jnp.where(l8[0:1, :] < 0.0, 0.0, m)
        p = jnp.exp2(buf[c * CK:(c + 1) * CK, :] - m)
        cl = jnp.sum(p.reshape(CK // 8, 8, BQ), axis=0)
        l8 = cl if l8 is None else l8 + cl
        oc = _dot(vat_ref[:, c * CK:(c + 1) * CK], p.astype(BF16))
        o = oc if o is None else o + oc
        return l8, o

    def a_finish(h, l8, o):
        off = pl.multiple_of(jnp.where(h < 0, D, h * DH), DH)
        ot_ref[pl.ds(off, DH), 0:BQ] = o / jnp.sum(l8, axis=0, keepdims=True)

    def a_body(j, carry, with_qk=True, extra=None):
        m_a, l8, o, m_b = carry
        pv_m = {-2: m_a, -1: m_b}
        m8 = None
        qh = None
        nsteps = 2 * NCK if with_qk else NCK + KA
        for s in range(nsteps):
            if with_qk:
                hq, cq = divmod(s, NCK)
                if cq == 0:
                    qh = qt_ref[pl.ds(pl.multiple_of((2 * j + hq) * DH, DH), DH), :]
                    m8 = None
                m8 = qk_chunk(qh, bufs[hq % 2], cq, m8)
                if cq == NCK - 1:
                    pv_m[hq] = jnp.max(m8, axis=0, keepdims=True)
            if extra is not None:
                extra(s)
            hp, cp = divmod(s - NCK - KA, NCK)
            if cp == 0:
                l8, o = None, None
            l8, o = pv_chunk(bufs[hp % 2], cp, pv_m[hp], l8, o)
            if cp == NCK - 1:
                a_finish(2 * j + hp, l8, o)
        if with_qk:
            return pv_m[0], l8, o, pv_m[1]
        return None

    zrow = jnp.zeros((1, BQ), F32)
    carry = (zrow, jnp.ones((8, BQ), F32), jnp.zeros((DH, BQ), F32), zrow)
    carry = jax.lax.fori_loop(0, H // 2, a_body, carry)
    @pl.when(i == 0)
    def _():
        cp_woa.wait()
        cp_wqkvb.wait()
        cp_wob.wait()

    cp_xb.wait()

    rowgrp = jax.lax.broadcasted_iota(jnp.int32, (4 * DH, BQ), 0) // DH

    def b_qproj(g):
        qg = (_dot(xb_ref[...], wqkvb_ref[:, g * 4 * DH:(g + 1) * 4 * DH]) * SCALE).T
        for j in range(4):
            qmj = jnp.where(rowgrp == j, qg, 0.0).astype(BF16)
            for t in range(NT):
                qm_ref[g * 4 * DH:(g + 1) * 4 * DH, (4 * t + j) * QB:(4 * t + j + 1) * QB] = (
                    qmj[:, t * QB:(t + 1) * QB])

    def extra(s):
        if s % 2 == 0 and s // 2 < NG:
            b_qproj(s // 2)

    a_body(H // 2, carry, with_qk=False, extra=extra)

    oa = ot_ref[0:D, 0:BQ].T.astype(BF16)
    out_ref[:, 0:D] = _dot(oa, woa_ref[...]).astype(out_ref.dtype)

    xb = xb_ref[...]
    kb_ref[pl.ds(row0, BQ), :] = _dot(xb, wqkvb_ref[:, D:2 * D]).astype(BF16)
    vb = _dot(xb, wqkvb_ref[:, 2 * D:3 * D])
    vbt_ref[:, pl.ds(row0, BQ)] = vb.T.astype(BF16)

    d0 = (jax.lax.broadcasted_iota(jnp.int32, (QB, QB), 1)
          - jax.lax.broadcasted_iota(jnp.int32, (QB, QB), 0))

    def key_off(t, c):
        n = i * NT + t
        return n, pl.multiple_of(jnp.maximum(n - 2, 0) * QB + c * QB, QB)

    def b_qk_chunk(t, g, buf, c, m8):
        n, koff = key_off(t, c)
        toff = pl.multiple_of(t * 4 * QB, 4 * QB)
        diff = d0 + (n * QB - koff)
        mask1 = diff.astype(jnp.uint32) < W
        mask = jnp.concatenate([mask1] * 4, axis=1)
        kc = kb_ref[pl.ds(koff, QB), g * 4 * DH:(g + 1) * 4 * DH]
        s = _dot(kc, qm_ref[g * 4 * DH:(g + 1) * 4 * DH, pl.ds(toff, 4 * QB)])
        s = jnp.where(mask, s, NEG)
        buf[c * QB:(c + 1) * QB, :] = s
        cm = jnp.max(s.reshape(QB // 8, 8, 4 * QB), axis=0)
        return cm if m8 is None else jnp.maximum(m8, cm)

    def b_pv_chunk(t, g, buf, c, m, l8, os_):
        n, koff = key_off(t, c)
        p = jnp.exp2(buf[c * QB:(c + 1) * QB, :] - m)
        cl = jnp.sum(p.reshape(QB // 8, 8, 4 * QB), axis=0)
        l8 = cl if l8 is None else l8 + cl
        new_os = []
        for j in range(4):
            h = 4 * g + j
            oj = _dot(vbt_ref[h * DH:(h + 1) * DH, pl.ds(koff, QB)],
                      p[:, j * QB:(j + 1) * QB].astype(BF16))
            new_os.append(oj if os_ is None else os_[j] + oj)
        return l8, new_os

    def b_finish(t, g, l8, os_):
        l = jnp.sum(l8, axis=0, keepdims=True)
        toff = pl.multiple_of(jnp.maximum(t, 0) * QB, QB)
        for j in range(4):
            off = pl.multiple_of(jnp.where(t < 0, D, (4 * g + j) * DH), DH)
            ot_ref[pl.ds(off, DH), pl.ds(toff, QB)] = os_[j] / l[:, j * QB:(j + 1) * QB]

    def b_body(t, carry, with_qk=True):
        m_a, l8, os_, m_b = carry
        pv_m = {-2: m_a, -1: m_b}
        m8 = None
        nsteps = NG * NC if with_qk else NC + KB
        for s in range(nsteps):
            if with_qk:
                gq, cq = divmod(s, NC)
                if cq == 0:
                    m8 = None
                m8 = b_qk_chunk(t, gq, bufs[gq % 2], cq, m8)
                if cq == NC - 1:
                    pv_m[gq] = jnp.max(m8, axis=0, keepdims=True)
            gp, cp = divmod(s - NC - KB, NC)
            tp, gg = (t - 1, gp + NG) if gp < 0 else (t, gp)
            if cp == 0:
                l8, os_ = None, None
            l8, os_ = b_pv_chunk(tp, gg, bufs[gp % 2], cp, pv_m[gp], l8, os_)
            if cp == NC - 1:
                b_finish(tp, gg, l8, os_)
        if with_qk:
            return pv_m[NG - 2], l8, os_, pv_m[NG - 1]
        return None

    zb = jnp.zeros((1, 4 * QB), F32)
    carry = (zb, jnp.ones((8, 4 * QB), F32), [jnp.zeros((DH, QB), F32)] * 4, zb)
    carry = jax.lax.fori_loop(0, NT, b_body, carry)
    b_body(NT, carry, with_qk=False)

    ob = ot_ref[0:D, 0:BQ].T.astype(BF16)
    out_ref[:, D:2 * D] = _dot(ob, wob_ref[...]).astype(out_ref.dtype)


@jax.jit
def pallas_concat_heads__grouped_kv_mqa__sliding_block__prompt_kernel(
    A_x: jax.Array,
    A_wq: jax.Array,
    A_wk: jax.Array,
    A_wv: jax.Array,
    A_wo: jax.Array,
    B_x: jax.Array,
    B_wqkv: jax.Array,
    B_wo: jax.Array,
):
    xa = A_x.reshape(S, D)
    xb = B_x.reshape(S, D)
    wkva = jnp.pad(jnp.concatenate([A_wk, A_wv], axis=1), ((0, 0), (0, 128 - 2 * DH)))

    hbm = pl.BlockSpec(memory_space=pl.ANY)
    out = pl.pallas_call(
        _kernel,
        grid=(S // BQ,),
        in_specs=[hbm] * 7,
        out_specs=pl.BlockSpec((BQ, 2 * D), lambda i: (i, 0)),
        out_shape=jax.ShapeDtypeStruct((S, 2 * D), BF16),
        scratch_shapes=[
            pltpu.VMEM((S, D), BF16),
            pltpu.VMEM((D, D), BF16),
            pltpu.VMEM((D, 128), BF16),
            pltpu.VMEM((D, D), BF16),
            pltpu.VMEM((BQ, D), BF16),
            pltpu.VMEM((D, 3 * D), BF16),
            pltpu.VMEM((D, D), BF16),
            pltpu.SemaphoreType.DMA((8,)),
            pltpu.VMEM((S, DH), BF16),
            pltpu.VMEM((DH, S), BF16),
            pltpu.VMEM((D, BQ), BF16),
            pltpu.VMEM((D + DH, BQ), F32),
            pltpu.VMEM((S, BQ), F32),
            pltpu.VMEM((S, BQ), F32),
            pltpu.VMEM((S, D), BF16),
            pltpu.VMEM((D, S), BF16),
            pltpu.VMEM((D, 4 * BQ), BF16),
        ],
        compiler_params=pltpu.CompilerParams(
            dimension_semantics=("arbitrary",),
            vmem_limit_bytes=100 * 1024 * 1024,
        ),
    )(xa, A_wq, wkva, A_wo, xb, B_wqkv, B_wo)
    return out.reshape(1, S, 2 * D)
```

```python
import math

import jax
import jax.numpy as jnp
import jax.experimental.pallas as pl
import jax.experimental.pallas.tpu as pltpu

S = 2048
D = 1024
H = 32
DH = 32
W = 256
BQ = 512
CK = 128
NCK = S // CK
QB = 128
KW = W + QB
NC = KW // QB
NG = H // 4
NT = BQ // QB
KA = 2
KB = 2
HB = 4
PACE = 2
BPACE = 2
SCALE = (DH ** -0.5) * math.log2(math.e)
NEG = -1e30

F32 = jnp.float32
BF16 = jnp.bfloat16


def _dot(a, b):
    return jnp.dot(a, b, preferred_element_type=F32)


def _kernel(xa_hbm, wqa_hbm, wkva_hbm, woa_hbm, xb_hbm, wqkvb_hbm, wob_hbm,
            out_ref,
            xa_ref, wqa_ref, wkva_ref, woa_ref, xb_ref, wqkvb_ref, wob_ref, sems,
            ka_ref, vat_ref, qt_ref, ot_ref, sa_ref, sb_ref, kb_ref, vbt_ref, qm_ref):
    i = pl.program_id(0)
    row0 = pl.multiple_of(i * BQ, BQ)
    bufs = (sa_ref, sb_ref)

    cp_xa0 = pltpu.make_async_copy(xa_hbm.at[0:BQ, :], xa_ref.at[0:BQ, :], sems.at[0])
    cp_wqa = pltpu.make_async_copy(wqa_hbm, wqa_ref, sems.at[1])
    cp_xa1 = pltpu.make_async_copy(xa_hbm.at[BQ:S, :], xa_ref.at[BQ:S, :], sems.at[2])
    cp_wkva = pltpu.make_async_copy(wkva_hbm, wkva_ref, sems.at[3])
    cp_woa = pltpu.make_async_copy(woa_hbm, woa_ref, sems.at[4])
    cp_wqkvb = pltpu.make_async_copy(wqkvb_hbm, wqkvb_ref, sems.at[5])
    cp_wob = pltpu.make_async_copy(wob_hbm, wob_ref, sems.at[6])
    cp_xb = pltpu.make_async_copy(xb_hbm.at[pl.ds(row0, BQ), :], xb_ref, sems.at[7])

    @pl.when(i == 0)
    def _():
        cp_xa0.start()
        cp_wqa.start()
        cp_xa1.start()
        cp_wkva.start()
        cp_woa.start()

    cp_xb.start()

    @pl.when(i == 0)
    def _():
        cp_wqkvb.start()
        cp_wob.start()
        def zfill(r, c):
            roff = pl.multiple_of(r * 256, 256)
            sa_ref[pl.ds(roff, 256), :] = jnp.zeros((256, BQ), F32)
            sb_ref[pl.ds(roff, 256), :] = jnp.zeros((256, BQ), F32)
            return c
        jax.lax.fori_loop(0, S // 256, zfill, 0)
        cp_xa0.wait()
        cp_wqa.wait()

    q = _dot(xa_ref[pl.ds(row0, BQ), :], wqa_ref[...]) * SCALE
    qt_ref[...] = q.T.astype(BF16)

    @pl.when(i == 0)
    def _():
        cp_xa1.wait()
        cp_wkva.wait()
        def kv_proj(r, c):
            roff = pl.multiple_of(r * 512, 512)
            kv = _dot(xa_ref[pl.ds(roff, 512), :], wkva_ref[...])
            ka_ref[pl.ds(roff, 512), :] = kv[:, 0:DH].astype(BF16)
            vat_ref[:, pl.ds(roff, 512)] = kv.T[DH:2 * DH, :].astype(BF16)
            return c
        jax.lax.fori_loop(0, S // 512, kv_proj, 0)

    def qk_chunk(qh, buf, c, m8):
        s = _dot(ka_ref[c * CK:(c + 1) * CK, :], qh)
        buf[c * CK:(c + 1) * CK, :] = s
        cm = jnp.max(s.reshape(CK // 8, 8, BQ), axis=0)
        return cm if m8 is None else jnp.maximum(m8, cm)

    def pv_chunk(buf, c, m, l8, o, pace=None):
        if pace is not None:
            m = jnp.where(pace[0:1, :] < -jnp.inf, 0.0, m)
        if l8 is not None:
            m = jnp.where(l8[0:1, :] < 0.0, 0.0, m)
        p = jnp.exp2(buf[c * CK:(c + 1) * CK, :] - m)
        cl = jnp.sum(p.reshape(CK // 8, 8, BQ), axis=0)
        l8 = cl if l8 is None else l8 + cl
        oc = _dot(vat_ref[:, c * CK:(c + 1) * CK], p.astype(BF16))
        o = oc if o is None else o + oc
        return l8, o

    def a_finish(h, l8, o):
        off = pl.multiple_of(jnp.where(h < 0, D, h * DH), DH)
        ot_ref[pl.ds(off, DH), 0:BQ] = o / jnp.sum(l8, axis=0, keepdims=True)

    def a_body(j, carry, with_qk=True, extra=None):
        m_a, l8, o, m_b = carry
        pv_m = {-2: m_a, -1: m_b}
        m8 = None
        qh = None
        hist = []
        nsteps = HB * NCK if with_qk else NCK + KA
        for s in range(nsteps):
            if with_qk:
                hq, cq = divmod(s, NCK)
                if cq == 0:
                    qh = qt_ref[pl.ds(pl.multiple_of((HB * j + hq) * DH, DH), DH), :]
                    m8 = None
                m8 = qk_chunk(qh, bufs[hq % 2], cq, m8)
                hist.append(m8)
                if cq == NCK - 1:
                    pv_m[hq] = jnp.max(m8, axis=0, keepdims=True)
            if extra is not None:
                extra(s)
            hp, cp = divmod(s - NCK - KA, NCK)
            if cp == 0:
                l8, o = None, None
            pace = hist[s - PACE] if (with_qk and s >= PACE) else None
            l8, o = pv_chunk(bufs[hp % 2], cp, pv_m[hp], l8, o, pace)
            if cp == NCK - 1:
                a_finish(HB * j + hp, l8, o)
        if with_qk:
            return pv_m[HB - 2], l8, o, pv_m[HB - 1]
        return None

    zrow = jnp.zeros((1, BQ), F32)
    carry = (zrow, jnp.ones((8, BQ), F32), jnp.zeros((DH, BQ), F32), zrow)
    carry = jax.lax.fori_loop(0, H // HB, a_body, carry)
    @pl.when(i == 0)
    def _():
        cp_woa.wait()
        cp_wqkvb.wait()
        cp_wob.wait()

    cp_xb.wait()

    rowgrp = jax.lax.broadcasted_iota(jnp.int32, (4 * DH, BQ), 0) // DH

    def b_qproj(g):
        qg = (_dot(xb_ref[...], wqkvb_ref[:, g * 4 * DH:(g + 1) * 4 * DH]) * SCALE).T
        for j in range(4):
            qmj = jnp.where(rowgrp == j, qg, 0.0).astype(BF16)
            for t in range(NT):
                qm_ref[g * 4 * DH:(g + 1) * 4 * DH, (4 * t + j) * QB:(4 * t + j + 1) * QB] = (
                    qmj[:, t * QB:(t + 1) * QB])

    def extra(s):
        if s % 2 == 0 and s // 2 < NG:
            b_qproj(s // 2)

    a_body(H // HB, carry, with_qk=False, extra=extra)

    oa = ot_ref[0:D, 0:BQ].T.astype(BF16)
    out_ref[:, 0:D] = _dot(oa, woa_ref[...]).astype(out_ref.dtype)

    xb = xb_ref[...]
    kb_ref[pl.ds(row0, BQ), :] = _dot(xb, wqkvb_ref[:, D:2 * D]).astype(BF16)
    vb = _dot(xb, wqkvb_ref[:, 2 * D:3 * D])
    vbt_ref[:, pl.ds(row0, BQ)] = vb.T.astype(BF16)

    d0 = (jax.lax.broadcasted_iota(jnp.int32, (QB, QB), 1)
          - jax.lax.broadcasted_iota(jnp.int32, (QB, QB), 0))

    def key_off(t, c):
        n = i * NT + t
        return n, pl.multiple_of(jnp.maximum(n - 2, 0) * QB + c * QB, QB)

    def b_qk_chunk(t, g, buf, c, m8):
        n, koff = key_off(t, c)
        toff = pl.multiple_of(t * 4 * QB, 4 * QB)
        diff = d0 + (n * QB - koff)
        mask1 = diff.astype(jnp.uint32) < W
        mask = jnp.concatenate([mask1] * 4, axis=1)
        kc = kb_ref[pl.ds(koff, QB), g * 4 * DH:(g + 1) * 4 * DH]
        s = _dot(kc, qm_ref[g * 4 * DH:(g + 1) * 4 * DH, pl.ds(toff, 4 * QB)])
        s = jnp.where(mask, s, NEG)
        buf[c * QB:(c + 1) * QB, :] = s
        cm = jnp.max(s.reshape(QB // 8, 8, 4 * QB), axis=0)
        return cm if m8 is None else jnp.maximum(m8, cm)

    def b_pv_chunk(t, g, buf, c, m, l8, os_, pace=None):
        n, koff = key_off(t, c)
        if pace is not None:
            m = jnp.where(pace[0:1, :] < -jnp.inf, 0.0, m)
        p = jnp.exp2(buf[c * QB:(c + 1) * QB, :] - m)
        cl = jnp.sum(p.reshape(QB // 8, 8, 4 * QB), axis=0)
        l8 = cl if l8 is None else l8 + cl
        new_os = []
        for j in range(4):
            h = 4 * g + j
            oj = _dot(vbt_ref[h * DH:(h + 1) * DH, pl.ds(koff, QB)],
                      p[:, j * QB:(j + 1) * QB].astype(BF16))
            new_os.append(oj if os_ is None else os_[j] + oj)
        return l8, new_os

    def b_finish(t, g, l8, os_):
        l = jnp.sum(l8, axis=0, keepdims=True)
        toff = pl.multiple_of(jnp.maximum(t, 0) * QB, QB)
        for j in range(4):
            off = pl.multiple_of(jnp.where(t < 0, D, (4 * g + j) * DH), DH)
            ot_ref[pl.ds(off, DH), pl.ds(toff, QB)] = os_[j] / l[:, j * QB:(j + 1) * QB]

    def b_body(t, carry, with_qk=True):
        m_a, l8, os_, m_b = carry
        pv_m = {-2: m_a, -1: m_b}
        m8 = None
        hist = []
        nsteps = NG * NC if with_qk else NC + KB
        for s in range(nsteps):
            if with_qk:
                gq, cq = divmod(s, NC)
                if cq == 0:
                    m8 = None
                m8 = b_qk_chunk(t, gq, bufs[gq % 2], cq, m8)
                hist.append(m8)
                if cq == NC - 1:
                    pv_m[gq] = jnp.max(m8, axis=0, keepdims=True)
            gp, cp = divmod(s - NC - KB, NC)
            tp, gg = (t - 1, gp + NG) if gp < 0 else (t, gp)
            if cp == 0:
                l8, os_ = None, None
            pace = hist[s - BPACE] if (with_qk and s >= BPACE) else None
            l8, os_ = b_pv_chunk(tp, gg, bufs[gp % 2], cp, pv_m[gp], l8, os_, pace)
            if cp == NC - 1:
                b_finish(tp, gg, l8, os_)
        if with_qk:
            return pv_m[NG - 2], l8, os_, pv_m[NG - 1]
        return None

    zb = jnp.zeros((1, 4 * QB), F32)
    carry = (zb, jnp.ones((8, 4 * QB), F32), [jnp.zeros((DH, QB), F32)] * 4, zb)
    carry = jax.lax.fori_loop(0, NT, b_body, carry)
    b_body(NT, carry, with_qk=False)

    ob = ot_ref[0:D, 0:BQ].T.astype(BF16)
    out_ref[:, D:2 * D] = _dot(ob, wob_ref[...]).astype(out_ref.dtype)


@jax.jit
def pallas_concat_heads__grouped_kv_mqa__sliding_block__prompt_kernel(
    A_x: jax.Array,
    A_wq: jax.Array,
    A_wk: jax.Array,
    A_wv: jax.Array,
    A_wo: jax.Array,
    B_x: jax.Array,
    B_wqkv: jax.Array,
    B_wo: jax.Array,
):
    xa = A_x.reshape(S, D)
    xb = B_x.reshape(S, D)
    wkva = jnp.pad(jnp.concatenate([A_wk, A_wv], axis=1), ((0, 0), (0, 128 - 2 * DH)))

    hbm = pl.BlockSpec(memory_space=pl.ANY)
    out = pl.pallas_call(
        _kernel,
        grid=(S // BQ,),
        in_specs=[hbm] * 7,
        out_specs=pl.BlockSpec((BQ, 2 * D), lambda i: (i, 0)),
        out_shape=jax.ShapeDtypeStruct((S, 2 * D), BF16),
        scratch_shapes=[
            pltpu.VMEM((S, D), BF16),
            pltpu.VMEM((D, D), BF16),
            pltpu.VMEM((D, 128), BF16),
            pltpu.VMEM((D, D), BF16),
            pltpu.VMEM((BQ, D), BF16),
            pltpu.VMEM((D, 3 * D), BF16),
            pltpu.VMEM((D, D), BF16),
            pltpu.SemaphoreType.DMA((8,)),
            pltpu.VMEM((S, DH), BF16),
            pltpu.VMEM((DH, S), BF16),
            pltpu.VMEM((D, BQ), BF16),
            pltpu.VMEM((D + DH, BQ), F32),
            pltpu.VMEM((S, BQ), F32),
            pltpu.VMEM((S, BQ), F32),
            pltpu.VMEM((S, D), BF16),
            pltpu.VMEM((D, S), BF16),
            pltpu.VMEM((D, 4 * BQ), BF16),
        ],
        compiler_params=pltpu.CompilerParams(
            dimension_semantics=("arbitrary",),
            vmem_limit_bytes=100 * 1024 * 1024,
        ),
    )(xa, A_wq, wkva, A_wo, xb, B_wqkv, B_wo)
    return out.reshape(1, S, 2 * D)
```
